```python
import os as _os
_os.environ.setdefault("JAX_PLATFORMS", "cpu")
import jax
import jax.numpy as jnp

def _softmax(x, axis=-1):
    return jax.nn.softmax(x, axis=axis)
def _gelu(x):
    return jax.nn.gelu(x, approximate=True)
def _silu(x):
    return jax.nn.silu(x)
def _sigmoid(x):
    return jax.nn.sigmoid(x)
def _layernorm(x, axis=-1, eps=1e-5):
    m = jnp.mean(x, axis=axis, keepdims=True)
    v = jnp.var(x, axis=axis, keepdims=True)
    return (x - m) / jnp.sqrt(v + eps)
def _scatter_add(tgt, idx, src, axis=0):
    return tgt.at[idx].add(src)
def _segment_sum(src, seg, n):
    return jax.ops.segment_sum(src, seg, n)
class _Rng:
    def __init__(self, key):
        self._k = key
    def _next(self):
        self._k, sub = jax.random.split(self._k)
        return sub
    def normal(self, shape):
        return jax.random.normal(self._next(), shape, dtype=jnp.bfloat16)
    def randint(self, lo, hi, shape):
        return jax.random.randint(self._next(), shape, lo, hi, dtype=jnp.int32)
    def uniform(self, shape, lo=0.0, hi=1.0):
        return jax.random.uniform(self._next(), shape, jnp.bfloat16, lo, hi)
    def permutation(self, n):
        return jax.random.permutation(self._next(), n)


kernel_name = 'standalone__mha_softmax__near_ridge'

def setup_inputs():
    _rng = _Rng(jax.random.key(int.from_bytes(__import__("os").urandom(4), "little")))
    _w = (lambda a: (lambda t: t.astype(jnp.bfloat16) if jnp.issubdtype(t.dtype, jnp.floating) else t)(jnp.asarray(a)))
    B, H, Sq, Sk, D = 8, 32, 496, 512, 192
    return {
        "q": _w((lambda *s: _rng.normal(s) * 0.05)(B, H, Sq, D)),
        "k": _w((lambda *s: _rng.normal(s) * 3.2)(B, H, Sk, D)),
        "v": _w((lambda *s: _rng.normal(s) * 0.05)(B, H, Sk, D)),
    }

def reference(q, k, v):
    scale = q.shape[-1] ** -0.5
    scores = jnp.einsum("bhqd,bhkd->bhqk", q, k) * scale
    p = _softmax(scores, axis=-1)
    return jnp.einsum("bhqk,bhkd->bhqd", p, v)
```

```python
import jax
import jax.numpy as jnp
import numpy as np
import jax.experimental.pallas as pl
import jax.experimental.pallas.tpu as pltpu

_HB = 8
_LOG2E = float(np.log2(np.e))


def _attn_kernel(qt_ref, kt_ref, vt_ref, ot_ref, *, hb, c):
    st, pp, ll = {}, {}, {}

    def scores(u):
        st[u] = jax.lax.dot_general(kt_ref[u], qt_ref[u], (((0,), (0,)), ((), ())),
                                    preferred_element_type=jnp.float32)

    def softmax(u):
        s = st.pop(u)
        m = jnp.max(s, axis=0, keepdims=True)
        p = jnp.exp2((s - m) * c)
        ll[u] = jnp.sum(p, axis=0, keepdims=True)
        pp[u] = p.astype(jnp.bfloat16)

    def output(u):
        ot = jnp.dot(vt_ref[u], pp.pop(u), preferred_element_type=jnp.float32)
        ot_ref[u] = (ot * (1.0 / ll.pop(u))).astype(ot_ref.dtype)

    for t in range(hb + 2):
        if t < hb:
            scores(t)
        if 0 <= t - 1 < hb:
            softmax(t - 1)
        if 0 <= t - 2 < hb:
            output(t - 2)


@jax.jit
def pallas_standalone__mha_softmax__near_ridge_kernel(
    q: jax.Array,
    k: jax.Array,
    v: jax.Array,
):
    B, H, Sq, D = q.shape
    Sk = k.shape[2]
    hb = _HB
    c = float(D ** -0.5) * _LOG2E
    qt = jnp.swapaxes(q, 2, 3).reshape(B * H, D, Sq)
    kt = jnp.swapaxes(k, 2, 3).reshape(B * H, D, Sk)
    vt = jnp.swapaxes(v, 2, 3).reshape(B * H, D, Sk)

    def kernel(qt_ref, kt_ref, vt_ref, ot_ref):
        _attn_kernel(qt_ref, kt_ref, vt_ref, ot_ref, hb=hb, c=c)

    ot = pl.pallas_call(
        kernel,
        grid=(B * H // hb,),
        in_specs=[
            pl.BlockSpec((hb, D, Sq), lambda i: (i, 0, 0)),
            pl.BlockSpec((hb, D, Sk), lambda i: (i, 0, 0)),
            pl.BlockSpec((hb, D, Sk), lambda i: (i, 0, 0)),
        ],
        out_specs=pl.BlockSpec((hb, D, Sq), lambda i: (i, 0, 0)),
        out_shape=jax.ShapeDtypeStruct((B * H, D, Sq), q.dtype),
        compiler_params=pltpu.CompilerParams(
            dimension_semantics=("parallel",),
            vmem_limit_bytes=100 * 1024 * 1024,
            flags={"XLA_TPU_FORCE_LP_LLO_SCHEDULER": True,
                   "XLA_TPU_EVENLY_DISTRIBUTE_CRITICAL_NODES": True},
        ),
    )(qt, kt, vt)
    return jnp.swapaxes(ot.reshape(B, H, D, Sq), 2, 3)
```

```python
import jax
import jax.numpy as jnp
import numpy as np
import jax.experimental.pallas as pl
import jax.experimental.pallas.tpu as pltpu

_G = 32
_DG = 2
_DGO = 2
_LOG2E = float(np.log2(np.e))


def _attention_kernel(q_hbm, k_hbm, v_hbm, o_hbm, qo, kb, vb, sq, sk, sv, so, *,
                      nh, g_size, dg, dgo, c):
    G = g_size
    sq_len = q_hbm.shape[2]
    n_groups = nh // G
    nd, no = G // dg, G // dgo

    def copy_in(kind, h, half, j):
        rows = pl.ds(j * dg, dg)
        if kind == "q":
            return pltpu.make_async_copy(q_hbm.at[pl.ds(h, dg)], qo.at[half, rows], sq.at[half * nd + j])
        if kind == "k":
            return pltpu.make_async_copy(k_hbm.at[pl.ds(h, dg)], kb.at[half, rows], sk.at[half * nd + j])
        return pltpu.make_async_copy(v_hbm.at[pl.ds(h, dg)], vb.at[half, rows], sv.at[half * nd + j])

    def copy_out(h, half, j):
        return pltpu.make_async_copy(qo.at[2 + half, pl.ds(j * dgo, dgo)], o_hbm.at[pl.ds(h, dgo)],
                                     so.at[half * no + j])

    for j in range(nd):
        for kind in "qkv":
            copy_in(kind, j * dg, 0, j).start()

    def body(g, carry):
        half = jax.lax.rem(g, 2)
        h0 = g * G
        has_next = g + 1 < n_groups

        @pl.when(g >= 2)
        def _():
            @pl.loop(0, no)
            def _(j):
                copy_out(0, half, j).wait()

        scores, probs, denom, q_val = {}, {}, {}, {}
        waited = set()

        def wait(kind, u):
            j = u // dg
            if (kind, j) not in waited:
                waited.add((kind, j))
                copy_in(kind, 0, half, j).wait()

        def prefetch(kind, j):
            @pl.when(has_next)
            def _():
                copy_in(kind, h0 + G + j * dg, 1 - half, j).start()

        def load_q(u):
            if 0 <= u < G and u not in q_val:
                wait("q", u)
                q_val[u] = qo[half, u]

        def score(u):
            load_q(u)
            wait("k", u)
            kt = kb[half, u]
            scores[u] = jax.lax.dot_general(q_val.pop(u), kt, (((0,), (0,)), ((), ())),
                                            preferred_element_type=jnp.float32)
            if u % dg == 0:
                prefetch("q", u // dg)
                prefetch("k", u // dg)

        def softmax(u):
            s = scores.pop(u)
            m = jnp.max(s, axis=1, keepdims=True)
            p = jnp.exp2((s - m) * c)
            l = jnp.sum(p, axis=1, keepdims=True)
            denom[u] = jnp.broadcast_to(l, (sq_len, 128)).T[0:1, :]
            probs[u] = p.astype(jnp.bfloat16)

        def output(u):
            wait("v", u)
            vt = vb[half, u]
            ot = jax.lax.dot_general(vt, probs.pop(u), (((1,), (1,)), ((), ())),
                                     preferred_element_type=jnp.float32)
            qo[2 + half, u] = (ot * (1.0 / denom.pop(u))).astype(qo.dtype)
            if u % dgo == dgo - 1:
                copy_out(h0 + u - (dgo - 1), half, u // dgo).start()
            if u % dg == 0:
                prefetch("v", u // dg)

        for t in range(G + 2):
            if t < G:
                score(t)
            load_q(t + 1)
            if 0 <= t - 1 < G:
                softmax(t - 1)
            if 0 <= t - 2 < G:
                output(t - 2)
        return carry

    jax.lax.fori_loop(0, n_groups, body, 0)
    for g in (n_groups - 2, n_groups - 1):
        for j in range(no):
            copy_out(0, g % 2, j).wait()


@jax.jit
def pallas_standalone__mha_softmax__near_ridge_kernel(
    q: jax.Array,
    k: jax.Array,
    v: jax.Array,
):
    B, H, Sq, D = q.shape
    Sk = k.shape[2]
    nh = B * H
    G, dg, dgo = _G, _DG, _DGO
    assert nh % G == 0 and nh // G >= 2 and G % dg == 0 and G % dgo == 0
    nd, no = G // dg, G // dgo

    qt = jnp.swapaxes(q, 2, 3).reshape(nh, D, Sq)
    kt = jnp.swapaxes(k, 2, 3).reshape(nh, D, Sk)
    vt = jnp.swapaxes(v, 2, 3).reshape(nh, D, Sk)

    def kernel(q_hbm, k_hbm, v_hbm, o_hbm, qo, kb, vb, sq, sk, sv, so):
        _attention_kernel(q_hbm, k_hbm, v_hbm, o_hbm, qo, kb, vb, sq, sk, sv, so,
                          nh=nh, g_size=G, dg=dg, dgo=dgo, c=float(D ** -0.5) * _LOG2E)

    ot = pl.pallas_call(
        kernel,
        in_specs=[pl.BlockSpec(memory_space=pl.ANY)] * 3,
        out_specs=pl.BlockSpec(memory_space=pl.ANY),
        out_shape=jax.ShapeDtypeStruct((nh, D, Sq), q.dtype),
        scratch_shapes=[
            pltpu.VMEM((4, G, D, Sq), q.dtype),
            pltpu.VMEM((2, G, D, Sk), k.dtype),
            pltpu.VMEM((2, G, D, Sk), v.dtype),
            pltpu.SemaphoreType.DMA((2 * nd,)),
            pltpu.SemaphoreType.DMA((2 * nd,)),
            pltpu.SemaphoreType.DMA((2 * nd,)),
            pltpu.SemaphoreType.DMA((2 * no,)),
        ],
        compiler_params=pltpu.CompilerParams(
            vmem_limit_bytes=100 * 1024 * 1024,
            disable_bounds_checks=True,
            flags={"XLA_TPU_RESCHEDULE_DMA_DONES": True},
        ),
    )(qt, kt, vt)
    return jnp.swapaxes(ot.reshape(B, H, D, Sq), 2, 3)
```

```python
import jax
import jax.numpy as jnp
import numpy as np
import jax.experimental.pallas as pl
import jax.experimental.pallas.tpu as pltpu

_G = 32
_IN_CHUNKS = (2,) * 16
_OUT_CHUNKS = (6, 6, 6, 6, 4, 2, 1, 1)
_LOG2E = float(np.log2(np.e))


def _chunk_tables(sizes):
    starts = [0]
    for n in sizes[:-1]:
        starts.append(starts[-1] + n)
    index = [c for c, n in enumerate(sizes) for _ in range(n)]
    return starts, index


def _attention_kernel(q_hbm, k_hbm, v_hbm, o_hbm, qo, kb, vb, q_next, sq, sk, sv, so, *,
                      nh, c):
    G = _G
    s_q = q_hbm.shape[2]
    s_k = k_hbm.shape[2]
    n_groups = nh // G
    in_start, in_index = _chunk_tables(_IN_CHUNKS)
    out_start, out_index = _chunk_tables(_OUT_CHUNKS)
    n_in = len(_IN_CHUNKS)

    def copy_in(kind, h0, half, j):
        s0, n = in_start[j], _IN_CHUNKS[j]
        rows = pl.ds(s0, n)
        if kind == "q":
            return pltpu.make_async_copy(q_hbm.at[pl.ds(h0 + s0, n)], qo.at[half, rows],
                                         sq.at[half * n_in + j])
        if kind == "k":
            return pltpu.make_async_copy(k_hbm.at[pl.ds(h0 + s0, n)], kb.at[half, rows],
                                         sk.at[half * n_in + j])
        return pltpu.make_async_copy(v_hbm.at[pl.ds(h0 + s0, n)], vb.at[half, rows],
                                     sv.at[half * n_in + j])

    def copy_out(h0, half, j):
        s0, n = out_start[j], _OUT_CHUNKS[j]
        return pltpu.make_async_copy(qo.at[2 + half, pl.ds(s0, n)], o_hbm.at[pl.ds(h0 + s0, n)],
                                     so.at[half])

    def wait_all_out(half):
        buf = qo.at[2 + half]
        pltpu.make_async_copy(buf, buf, so.at[half]).wait()

    first = [("q", 0), ("k", 0), ("v", 0), ("q", 1), ("k", 1), ("k", 2), ("q", 2), ("v", 1)]
    need = [(in_start[j], 0, kind, j) for kind in "qk" for j in range(n_in)]
    need += [(in_start[j] + 2.5, 1, "v", j) for j in range(n_in)]
    rest = [(kind, j) for _, _, kind, j in sorted(need)]
    for kind, j in first + [x for x in rest if x not in first]:
        copy_in(kind, 0, 0, j).start()

    def body(g, carry):
        half = jax.lax.rem(g, 2)
        other = 1 - half
        h0 = g * G
        has_next = g + 1 < n_groups

        @pl.when(g == 0)
        def _():
            copy_in("q", 0, 0, 0).wait()
            q_next[...] = qo[0, 0].T

        @pl.when(g >= 2)
        def _():
            wait_all_out(half)

        scores, maxes, probs, denom, q_val = {}, {}, {}, {}, {}
        waited = {("q", 0)}

        def wait(kind, u):
            j = in_index[u]
            if (kind, j) not in waited:
                waited.add((kind, j))
                copy_in(kind, 0, half, j).wait()

        def prefetch(kind, u):
            if u in in_start:
                @pl.when(has_next)
                def _():
                    copy_in(kind, h0 + G, other, in_index[u]).start()

        def load_q(u):
            if 0 <= u < G and u not in q_val:
                wait("q", u)
                q_val[u] = qo[half, u]

        def score(u):
            wait("k", u)
            if u == 0:
                scores[u] = jnp.dot(q_next[...], kb[half, u], preferred_element_type=jnp.float32)
            else:
                load_q(u)
                q_t = q_val.pop(u)
                scores[u] = jax.lax.dot_general(q_t, kb[half, u], (((0,), (0,)), ((), ())),
                                                preferred_element_type=jnp.float32)
            prefetch("q", u)
            prefetch("k", u)

        def row_max(u):
            t = [scores[u][:, 128 * j:128 * (j + 1)] for j in range(s_k // 128)]
            r = jnp.maximum(jnp.maximum(jnp.maximum(t[1], t[2]), t[0]), t[3])
            maxes[u] = jnp.max(r, axis=1, keepdims=True)

        def softmax(u):
            s = scores.pop(u)
            p = jnp.exp2((s - maxes.pop(u)) * c).astype(jnp.bfloat16)
            l = jnp.sum(p.astype(jnp.float32), axis=1, keepdims=True)
            denom[u] = jnp.broadcast_to(l, (s_q, 128)).T[0:1, :]
            probs[u] = p

        def output(u):
            wait("v", u)
            o_t = jax.lax.dot_general(vb[half, u], probs.pop(u), (((1,), (1,)), ((), ())),
                                      preferred_element_type=jnp.float32)
            qo[2 + half, u] = (o_t * (1.0 / denom.pop(u))).astype(qo.dtype)
            if u + 1 == G or u + 1 in out_start:
                copy_out(h0, half, out_index[u]).start()
            prefetch("v", u)

        for t in range(G + 2):
            if t < G:
                score(t)
                row_max(t)
            load_q(t + 1)
            if 0 <= t - 1 < G:
                softmax(t - 1)
            if 0 <= t - 2 < G:
                output(t - 2)
            if t == G - 1:
                @pl.when(has_next)
                def _():
                    copy_in("q", 0, other, 0).wait()
                q_next[...] = qo[other, 0].T
        return carry

    jax.lax.fori_loop(0, n_groups, body, 0)
    for g in (n_groups - 2, n_groups - 1):
        wait_all_out(g % 2)


@jax.jit
def pallas_standalone__mha_softmax__near_ridge_kernel(
    q: jax.Array,
    k: jax.Array,
    v: jax.Array,
):
    B, H, Sq, D = q.shape
    Sk = k.shape[2]
    nh = B * H
    G = _G
    assert nh % G == 0 and nh // G >= 2 and Sk == 512
    assert sum(_IN_CHUNKS) == G and sum(_OUT_CHUNKS) == G
    n_in = len(_IN_CHUNKS)

    qt = jnp.swapaxes(q, 2, 3).reshape(nh, D, Sq)
    kt = jnp.swapaxes(k, 2, 3).reshape(nh, D, Sk)
    vt = jnp.swapaxes(v, 2, 3).reshape(nh, D, Sk)

    def kernel(q_hbm, k_hbm, v_hbm, o_hbm, qo, kb, vb, q_next, sq, sk, sv, so):
        _attention_kernel(q_hbm, k_hbm, v_hbm, o_hbm, qo, kb, vb, q_next, sq, sk, sv, so,
                          nh=nh, c=float(D ** -0.5) * _LOG2E)

    ot = pl.pallas_call(
        kernel,
        in_specs=[pl.BlockSpec(memory_space=pl.ANY)] * 3,
        out_specs=pl.BlockSpec(memory_space=pl.ANY),
        out_shape=jax.ShapeDtypeStruct((nh, D, Sq), q.dtype),
        scratch_shapes=[
            pltpu.VMEM((4, G, D, Sq), q.dtype),
            pltpu.VMEM((2, G, D, Sk), k.dtype),
            pltpu.VMEM((2, G, D, Sk), v.dtype),
            pltpu.VMEM((Sq, D), q.dtype),
            pltpu.SemaphoreType.DMA((2 * n_in,)),
            pltpu.SemaphoreType.DMA((2 * n_in,)),
            pltpu.SemaphoreType.DMA((2 * n_in,)),
            pltpu.SemaphoreType.DMA((2,)),
        ],
        compiler_params=pltpu.CompilerParams(
            vmem_limit_bytes=100 * 1024 * 1024,
            disable_bounds_checks=True,
            flags={"XLA_TPU_RESCHEDULE_DMA_DONES": True},
        ),
    )(qt, kt, vt)
    return jnp.swapaxes(ot.reshape(B, H, D, Sq), 2, 3)
```

```python
import jax
import jax.numpy as jnp
import numpy as np
import jax.experimental.pallas as pl
import jax.experimental.pallas.tpu as pltpu

_G = 32
_DG = 2
_OUT_CHUNKS = (6, 6, 6, 6, 4, 2, 1, 1)
_LOG2E = float(np.log2(np.e))


def _chunk_tables(sizes):
    starts = [0]
    for n in sizes[:-1]:
        starts.append(starts[-1] + n)
    index = [c for c, n in enumerate(sizes) for _ in range(n)]
    return starts, index


def _attention_kernel(q_hbm, k_hbm, v_hbm, o_hbm, qo, kb, vb, q_next, sq, sk, sv, so, *,
                      nh, c):
    G = _G
    s_q = q_hbm.shape[2]
    n_groups = nh // G
    dg = _DG
    n_in = G // dg
    out_start, out_index = _chunk_tables(_OUT_CHUNKS)

    def copy_in(kind, h0, half, j):
        s0, n = j * dg, dg
        rows = pl.ds(s0, n)
        if kind == "q":
            return pltpu.make_async_copy(q_hbm.at[pl.ds(h0 + s0, n)], qo.at[half, rows],
                                         sq.at[half * n_in + j])
        if kind == "k":
            return pltpu.make_async_copy(k_hbm.at[pl.ds(h0 + s0, n)], kb.at[half, rows],
                                         sk.at[half * n_in + j])
        return pltpu.make_async_copy(v_hbm.at[pl.ds(h0 + s0, n)], vb.at[half, rows],
                                     sv.at[half * n_in + j])

    def copy_out(h0, half, j):
        s0, n = out_start[j], _OUT_CHUNKS[j]
        return pltpu.make_async_copy(qo.at[2 + half, pl.ds(s0, n)], o_hbm.at[pl.ds(h0 + s0, n)],
                                     so.at[half])

    def wait_all_out(half):
        buf = qo.at[2 + half]
        pltpu.make_async_copy(buf, buf, so.at[half]).wait()

    @pl.loop(0, n_in + 1)
    def _(j):
        @pl.when(j < n_in)
        def _():
            rows = pl.ds(j * dg, dg)
            pltpu.make_async_copy(q_hbm.at[rows], qo.at[0, rows], sq.at[j]).start()
            pltpu.make_async_copy(k_hbm.at[rows], kb.at[0, rows], sk.at[j]).start()

        @pl.when(j >= 1)
        def _():
            rows = pl.ds((j - 1) * dg, dg)
            pltpu.make_async_copy(v_hbm.at[rows], vb.at[0, rows], sv.at[j - 1]).start()

    def body(g, carry):
        half = jax.lax.rem(g, 2)
        other = 1 - half
        h0 = g * G
        has_next = g + 1 < n_groups

        @pl.when(g == 0)
        def _():
            copy_in("q", 0, 0, 0).wait()
            q_next[...] = qo[0, 0].T

        @pl.when(g >= 2)
        def _():
            wait_all_out(half)

        scores, maxes, probs, denom, q_val = {}, {}, {}, {}, {}
        waited = {("q", 0)}

        def wait(kind, u):
            j = u // dg
            if (kind, j) not in waited:
                waited.add((kind, j))
                copy_in(kind, 0, half, j).wait()

        def prefetch(kind, u):
            if u % dg == 0:
                @pl.when(has_next)
                def _():
                    copy_in(kind, h0 + G, other, u // dg).start()

        def load_q(u):
            if 0 <= u < G and u not in q_val:
                wait("q", u)
                q_val[u] = qo[half, u]

        def score(u):
            wait("k", u)
            if u == 0:
                scores[u] = jnp.dot(q_next[...], kb[half, u], preferred_element_type=jnp.float32)
            else:
                load_q(u)
                q_t = q_val.pop(u)
                scores[u] = jax.lax.dot_general(q_t, kb[half, u], (((0,), (0,)), ((), ())),
                                                preferred_element_type=jnp.float32)
            prefetch("q", u)
            prefetch("k", u)

        def row_max(u):
            t = [scores[u][:, 128 * j:128 * (j + 1)] for j in range(4)]
            r = jnp.maximum(jnp.maximum(jnp.maximum(t[1], t[2]), t[0]), t[3])
            maxes[u] = jnp.max(r, axis=1, keepdims=True)

        def softmax(u):
            s, m = scores.pop(u), maxes.pop(u)
            e = {}
            for j in (2, 3, 0, 1):
                e[j] = jnp.exp2((s[:, 128 * j:128 * (j + 1)] - m) * c)
            p = jnp.concatenate([e[j] for j in range(4)], axis=1).astype(jnp.bfloat16)
            l = jnp.sum(p.astype(jnp.float32), axis=1, keepdims=True)
            denom[u] = jnp.broadcast_to(l, (s_q, 128)).T[0:1, :]
            probs[u] = p

        def output(u):
            wait("v", u)
            o_t = jax.lax.dot_general(vb[half, u], probs.pop(u), (((1,), (1,)), ((), ())),
                                      preferred_element_type=jnp.float32)
            qo[2 + half, u] = (o_t * (1.0 / denom.pop(u))).astype(qo.dtype)
            if u + 1 == G or u + 1 in out_start:
                copy_out(h0, half, out_index[u]).start()
            prefetch("v", u)

        for t in range(G + 2):
            if t < G:
                score(t)
                row_max(t)
            load_q(t + 1)
            if 0 <= t - 1 < G:
                softmax(t - 1)
            if 0 <= t - 2 < G:
                output(t - 2)
            if t == G - 1:
                @pl.when(has_next)
                def _():
                    copy_in("q", 0, other, 0).wait()
                q_next[...] = qo[other, 0].T
        return carry

    jax.lax.fori_loop(0, n_groups, body, 0)
    for g in (n_groups - 2, n_groups - 1):
        wait_all_out(g % 2)


@jax.jit
def pallas_standalone__mha_softmax__near_ridge_kernel(
    q: jax.Array,
    k: jax.Array,
    v: jax.Array,
):
    B, H, Sq, D = q.shape
    Sk = k.shape[2]
    nh = B * H
    G = _G
    assert nh % G == 0 and nh // G >= 2 and Sk == 512
    assert G % _DG == 0 and sum(_OUT_CHUNKS) == G
    n_in = G // _DG

    qt = jnp.swapaxes(q, 2, 3).reshape(nh, D, Sq)
    kt = jnp.swapaxes(k, 2, 3).reshape(nh, D, Sk)
    vt = jnp.swapaxes(v, 2, 3).reshape(nh, D, Sk)

    def kernel(q_hbm, k_hbm, v_hbm, o_hbm, qo, kb, vb, q_next, sq, sk, sv, so):
        _attention_kernel(q_hbm, k_hbm, v_hbm, o_hbm, qo, kb, vb, q_next, sq, sk, sv, so,
                          nh=nh, c=float(D ** -0.5) * _LOG2E)

    ot = pl.pallas_call(
        kernel,
        in_specs=[pl.BlockSpec(memory_space=pl.ANY)] * 3,
        out_specs=pl.BlockSpec(memory_space=pl.ANY),
        out_shape=jax.ShapeDtypeStruct((nh, D, Sq), q.dtype),
        scratch_shapes=[
            pltpu.VMEM((4, G, D, Sq), q.dtype),
            pltpu.VMEM((2, G, D, Sk), k.dtype),
            pltpu.VMEM((2, G, D, Sk), v.dtype),
            pltpu.VMEM((Sq, D), q.dtype),
            pltpu.SemaphoreType.DMA((2 * n_in,)),
            pltpu.SemaphoreType.DMA((2 * n_in,)),
            pltpu.SemaphoreType.DMA((2 * n_in,)),
            pltpu.SemaphoreType.DMA((2,)),
        ],
        compiler_params=pltpu.CompilerParams(
            vmem_limit_bytes=100 * 1024 * 1024,
            disable_bounds_checks=True,
            flags={"XLA_TPU_RESCHEDULE_DMA_DONES": True},
        ),
    )(qt, kt, vt)
    return jnp.swapaxes(ot.reshape(B, H, D, Sq), 2, 3)
```

```python
import jax
import jax.numpy as jnp
import numpy as np
import jax.experimental.pallas as pl
import jax.experimental.pallas.tpu as pltpu

_G = 32
_DG = 2
_LEAD = 4
_OUT_CHUNKS = (6, 6, 6, 6, 4, 2, 1, 1)
_LOG2E = float(np.log2(np.e))


def _chunk_tables(sizes):
    starts = [0]
    for n in sizes[:-1]:
        starts.append(starts[-1] + n)
    index = [c for c, n in enumerate(sizes) for _ in range(n)]
    return starts, index


def _attention_kernel(q_hbm, k_hbm, v_hbm, o_hbm, qo, kb, vb, q_next, sq, sk, sv, so, *,
                      nh, c):
    G = _G
    s_q = q_hbm.shape[2]
    n_groups = nh // G
    dg = _DG
    n_in = G // dg
    lead = _LEAD
    out_start, out_index = _chunk_tables(_OUT_CHUNKS)

    def copy_in(kind, h0, half, j, sem0=0):
        s0, n = j * dg, dg
        rows = pl.ds(s0, n)
        if kind == "q":
            return pltpu.make_async_copy(q_hbm.at[pl.ds(h0 + s0, n)], qo.at[half, rows],
                                         sq.at[j % lead])
        if kind == "k":
            return pltpu.make_async_copy(k_hbm.at[pl.ds(h0 + s0, n)], kb.at[half, rows],
                                         sk.at[j % lead])
        return pltpu.make_async_copy(v_hbm.at[pl.ds(h0 + s0, n)], vb.at[half, rows],
                                     sv.at[sem0 + j % lead])

    def copy_out(h0, half, j):
        s0, n = out_start[j], _OUT_CHUNKS[j]
        return pltpu.make_async_copy(qo.at[2 + half, pl.ds(s0, n)], o_hbm.at[pl.ds(h0 + s0, n)],
                                     so.at[half])

    def wait_all_out(half):
        buf = qo.at[2 + half]
        pltpu.make_async_copy(buf, buf, so.at[half]).wait()

    @pl.loop(0, lead + 1)
    def _(j):
        @pl.when(j < lead)
        def _():
            rows = pl.ds(j * dg, dg)
            pltpu.make_async_copy(q_hbm.at[rows], qo.at[0, rows], sq.at[j]).start()
            pltpu.make_async_copy(k_hbm.at[rows], kb.at[0, rows], sk.at[j]).start()

        @pl.when(j >= 1)
        def _():
            rows = pl.ds((j - 1) * dg, dg)
            pltpu.make_async_copy(v_hbm.at[rows], vb.at[0, rows], sv.at[j - 1]).start()

    def body(g, carry):
        half = jax.lax.rem(g, 2)
        other = 1 - half
        h0 = g * G
        has_next = g + 1 < n_groups
        v_sem0 = jax.lax.shift_right_logical(g, 20)

        @pl.when(g == 0)
        def _():
            copy_in("q", 0, 0, 0).wait()
            q_next[...] = qo[0, 0].T

        @pl.when(g >= 2)
        def _():
            wait_all_out(half)

        scores, maxes, probs, denom, q_val = {}, {}, {}, {}, {}
        waited = {("q", 0)}

        def wait(kind, u):
            j = u // dg
            if (kind, j) not in waited:
                waited.add((kind, j))
                copy_in(kind, 0, half, j, v_sem0).wait()

        def prefetch(kind, u):
            if u % dg:
                return
            j = u // dg + lead
            if j < n_in:
                copy_in(kind, h0, half, j, v_sem0).start()
            else:
                @pl.when(has_next)
                def _():
                    copy_in(kind, h0 + G, other, j - n_in, v_sem0).start()

        def load_q(u):
            if 0 <= u < G and u not in q_val:
                wait("q", u)
                q_val[u] = qo[half, u]

        def score(u):
            wait("k", u)
            if u == 0:
                scores[u] = jnp.dot(q_next[...], kb[half, u], preferred_element_type=jnp.float32)
            else:
                load_q(u)
                q_t = q_val.pop(u)
                scores[u] = jax.lax.dot_general(q_t, kb[half, u], (((0,), (0,)), ((), ())),
                                                preferred_element_type=jnp.float32)
            prefetch("q", u)
            prefetch("k", u)

        def row_max(u):
            t = [scores[u][:, 128 * j:128 * (j + 1)] for j in range(4)]
            r = jnp.maximum(jnp.maximum(jnp.maximum(t[1], t[2]), t[0]), t[3])
            maxes[u] = jnp.max(r, axis=1, keepdims=True)

        def softmax(u):
            s, m = scores.pop(u), maxes.pop(u)
            e = {}
            for j in (2, 3, 0, 1):
                e[j] = jnp.exp2((s[:, 128 * j:128 * (j + 1)] - m) * c)
            p = jnp.concatenate([e[j] for j in range(4)], axis=1).astype(jnp.bfloat16)
            l = jnp.sum(p.astype(jnp.float32), axis=1, keepdims=True)
            denom[u] = jnp.broadcast_to(l, (s_q, 128)).T[0:1, :]
            probs[u] = p

        def output(u):
            wait("v", u)
            o_t = jax.lax.dot_general(vb[half, u], probs.pop(u), (((1,), (1,)), ((), ())),
                                      preferred_element_type=jnp.float32)
            r = 1.0 / denom.pop(u)
            cols = [slice(a, min(a + 128, s_q)) for a in range(0, s_q, 128)]
            qo[2 + half, u] = jnp.concatenate(
                [(o_t[:, w] * r[:, w]).astype(qo.dtype) for w in cols], axis=1)
            if u + 1 == G or u + 1 in out_start:
                copy_out(h0, half, out_index[u]).start()
            prefetch("v", u)

        for t in range(G + 2):
            if t < G:
                score(t)
                row_max(t)
            load_q(t + 1)
            if 0 <= t - 1 < G:
                softmax(t - 1)
            if 0 <= t - 2 < G:
                output(t - 2)
            if t == G - 1:
                @pl.when(has_next)
                def _():
                    copy_in("q", 0, other, 0).wait()
                q_next[...] = qo[other, 0].T
        return carry

    jax.lax.fori_loop(0, n_groups, body, 0)
    for g in (n_groups - 2, n_groups - 1):
        wait_all_out(g % 2)


@jax.jit
def pallas_standalone__mha_softmax__near_ridge_kernel(
    q: jax.Array,
    k: jax.Array,
    v: jax.Array,
):
    B, H, Sq, D = q.shape
    Sk = k.shape[2]
    nh = B * H
    G = _G
    assert nh % G == 0 and nh // G >= 2 and Sk == 512
    assert G % _DG == 0 and (G // _DG) % _LEAD == 0 and sum(_OUT_CHUNKS) == G

    qt = jnp.swapaxes(q, 2, 3).reshape(nh, D, Sq)
    kt = jnp.swapaxes(k, 2, 3).reshape(nh, D, Sk)
    vt = jnp.swapaxes(v, 2, 3).reshape(nh, D, Sk)

    def kernel(q_hbm, k_hbm, v_hbm, o_hbm, qo, kb, vb, q_next, sq, sk, sv, so):
        _attention_kernel(q_hbm, k_hbm, v_hbm, o_hbm, qo, kb, vb, q_next, sq, sk, sv, so,
                          nh=nh, c=float(D ** -0.5) * _LOG2E)

    ot = pl.pallas_call(
        kernel,
        in_specs=[pl.BlockSpec(memory_space=pl.ANY)] * 3,
        out_specs=pl.BlockSpec(memory_space=pl.ANY),
        out_shape=jax.ShapeDtypeStruct((nh, D, Sq), q.dtype),
        scratch_shapes=[
            pltpu.VMEM((4, G, D, Sq), q.dtype),
            pltpu.VMEM((2, G, D, Sk), k.dtype),
            pltpu.VMEM((2, G, D, Sk), v.dtype),
            pltpu.VMEM((Sq, D), q.dtype),
            pltpu.SemaphoreType.DMA((_LEAD,)),
            pltpu.SemaphoreType.DMA((_LEAD,)),
            pltpu.SemaphoreType.DMA((_LEAD,)),
            pltpu.SemaphoreType.DMA((2,)),
        ],
        compiler_params=pltpu.CompilerParams(
            vmem_limit_bytes=80 * 1024 * 1024,
            disable_bounds_checks=True,
            flags={"XLA_TPU_RESCHEDULE_DMA_DONES": True},
        ),
    )(qt, kt, vt)
    return jnp.swapaxes(ot.reshape(B, H, D, Sq), 2, 3)
```

```python
import jax
import jax.numpy as jnp
import numpy as np
import jax.experimental.pallas as pl
import jax.experimental.pallas.tpu as pltpu

_G = 32
_DG = 2
_LEAD = 4
_OUT_CHUNKS = (6, 6, 6, 6, 4, 2, 1, 1)
_LAST_SPLIT = 384
_LOG2E = float(np.log2(np.e))


def _chunk_tables(sizes):
    starts = [0]
    for n in sizes[:-1]:
        starts.append(starts[-1] + n)
    index = [c for c, n in enumerate(sizes) for _ in range(n)]
    return starts, index


def _attention_kernel(q_hbm, k_hbm, v_hbm, o_hbm, qo, kb, vb, q_next, sq, sk, sv, so, *,
                      nh, c):
    G = _G
    s_q = q_hbm.shape[2]
    n_groups = nh // G
    dg = _DG
    n_in = G // dg
    lead = _LEAD
    out_start, out_index = _chunk_tables(_OUT_CHUNKS)

    def copy_in(kind, h0, half, j, sem0=0):
        s0, n = j * dg, dg
        rows = pl.ds(s0, n)
        if kind == "q":
            return pltpu.make_async_copy(q_hbm.at[pl.ds(h0 + s0, n)], qo.at[half, rows],
                                         sq.at[j % lead])
        if kind == "k":
            return pltpu.make_async_copy(k_hbm.at[pl.ds(h0 + s0, n)], kb.at[half, rows],
                                         sk.at[j % lead])
        return pltpu.make_async_copy(v_hbm.at[pl.ds(h0 + s0, n)], vb.at[half, rows],
                                     sv.at[sem0 + j % lead])

    def copy_out(h0, half, j):
        s0, n = out_start[j], _OUT_CHUNKS[j]
        return pltpu.make_async_copy(qo.at[2 + half, pl.ds(s0, n)], o_hbm.at[pl.ds(h0 + s0, n)],
                                     so.at[half])

    def wait_all_out(half):
        buf = qo.at[2 + half]
        pltpu.make_async_copy(buf, buf, so.at[half]).wait()

    @pl.loop(0, lead + 1)
    def _(j):
        @pl.when(j < lead)
        def _():
            rows = pl.ds(j * dg, dg)
            pltpu.make_async_copy(q_hbm.at[rows], qo.at[0, rows], sq.at[j]).start()
            pltpu.make_async_copy(k_hbm.at[rows], kb.at[0, rows], sk.at[j]).start()

        @pl.when(j >= 1)
        def _():
            rows = pl.ds((j - 1) * dg, dg)
            pltpu.make_async_copy(v_hbm.at[rows], vb.at[0, rows], sv.at[j - 1]).start()

    def body(g, carry):
        half = jax.lax.rem(g, 2)
        other = 1 - half
        h0 = g * G
        has_next = g + 1 < n_groups
        v_sem0 = jax.lax.shift_right_logical(g, 20)

        @pl.when(g == 0)
        def _():
            copy_in("q", 0, 0, 0).wait()
            q_next[...] = qo[0, 0].T

        @pl.when(g >= 2)
        def _():
            wait_all_out(half)

        scores, maxes, probs, denom, q_val = {}, {}, {}, {}, {}
        waited = {("q", 0)}

        def wait(kind, u):
            j = u // dg
            if (kind, j) not in waited:
                waited.add((kind, j))
                copy_in(kind, 0, half, j, v_sem0).wait()

        def prefetch(kind, u):
            if u % dg:
                return
            j = u // dg + lead
            if j < n_in:
                copy_in(kind, h0, half, j, v_sem0).start()
            else:
                @pl.when(has_next)
                def _():
                    copy_in(kind, h0 + G, other, j - n_in, v_sem0).start()

        def load_q(u):
            if 0 <= u < G and u not in q_val:
                wait("q", u)
                q_val[u] = qo[half, u]

        def score(u):
            wait("k", u)
            if u == 0:
                scores[u] = jnp.dot(q_next[...], kb[half, u], preferred_element_type=jnp.float32)
            else:
                load_q(u)
                q_t = q_val.pop(u)
                scores[u] = jax.lax.dot_general(q_t, kb[half, u], (((0,), (0,)), ((), ())),
                                                preferred_element_type=jnp.float32)
            prefetch("q", u)
            prefetch("k", u)

        def row_max(u):
            t = [scores[u][:, 128 * j:128 * (j + 1)] for j in range(4)]
            r = jnp.maximum(jnp.maximum(jnp.maximum(t[1], t[2]), t[0]), t[3])
            maxes[u] = jnp.max(r, axis=1, keepdims=True)

        def softmax(u):
            s, m = scores.pop(u), maxes.pop(u)
            e = {}
            for j in (2, 3, 0, 1):
                e[j] = jnp.exp2((s[:, 128 * j:128 * (j + 1)] - m) * c)
            p = jnp.concatenate([e[j] for j in range(4)], axis=1).astype(jnp.bfloat16)
            l = jnp.sum(p.astype(jnp.float32), axis=1, keepdims=True)
            denom[u] = jnp.broadcast_to(l, (s_q, 128)).T[0:1, :]
            probs[u] = p

        def output(u):
            wait("v", u)
            o_t = jax.lax.dot_general(vb[half, u], probs.pop(u), (((1,), (1,)), ((), ())),
                                      preferred_element_type=jnp.float32)
            r = 1.0 / denom.pop(u)
            cols = [slice(a, min(a + 128, s_q)) for a in range(0, s_q, 128)]
            o = jnp.concatenate([(o_t[:, w] * r[:, w]).astype(qo.dtype) for w in cols], axis=1)
            if u + 1 < G:
                qo[2 + half, u] = o
                if u + 1 in out_start:
                    copy_out(h0, half, out_index[u]).start()
            else:
                for lo, hi in ((0, _LAST_SPLIT), (_LAST_SPLIT, s_q)):
                    qo[2 + half, u, :, lo:hi] = o[:, lo:hi]
                    pltpu.make_async_copy(qo.at[2 + half, u, :, pl.ds(lo, hi - lo)],
                                          o_hbm.at[h0 + u, :, pl.ds(lo, hi - lo)],
                                          so.at[half]).start()
            prefetch("v", u)

        for t in range(G + 2):
            if t < G:
                score(t)
                row_max(t)
            load_q(t + 1)
            if 0 <= t - 1 < G:
                softmax(t - 1)
            if 0 <= t - 2 < G:
                output(t - 2)
            if t == G - 1:
                @pl.when(has_next)
                def _():
                    copy_in("q", 0, other, 0).wait()
                q_next[...] = qo[other, 0].T
        return carry

    jax.lax.fori_loop(0, n_groups, body, 0)
    for g in (n_groups - 2, n_groups - 1):
        wait_all_out(g % 2)


@jax.jit
def pallas_standalone__mha_softmax__near_ridge_kernel(
    q: jax.Array,
    k: jax.Array,
    v: jax.Array,
):
    B, H, Sq, D = q.shape
    Sk = k.shape[2]
    nh = B * H
    G = _G
    assert nh % G == 0 and nh // G >= 2 and Sk == 512
    assert G % _DG == 0 and (G // _DG) % _LEAD == 0 and sum(_OUT_CHUNKS) == G and _OUT_CHUNKS[-1] == 1

    qt = jnp.swapaxes(q, 2, 3).reshape(nh, D, Sq)
    kt = jnp.swapaxes(k, 2, 3).reshape(nh, D, Sk)
    vt = jnp.swapaxes(v, 2, 3).reshape(nh, D, Sk)

    def kernel(q_hbm, k_hbm, v_hbm, o_hbm, qo, kb, vb, q_next, sq, sk, sv, so):
        _attention_kernel(q_hbm, k_hbm, v_hbm, o_hbm, qo, kb, vb, q_next, sq, sk, sv, so,
                          nh=nh, c=float(D ** -0.5) * _LOG2E)

    ot = pl.pallas_call(
        kernel,
        in_specs=[pl.BlockSpec(memory_space=pl.ANY)] * 3,
        out_specs=pl.BlockSpec(memory_space=pl.ANY),
        out_shape=jax.ShapeDtypeStruct((nh, D, Sq), q.dtype),
        scratch_shapes=[
            pltpu.VMEM((4, G, D, Sq), q.dtype),
            pltpu.VMEM((2, G, D, Sk), k.dtype),
            pltpu.VMEM((2, G, D, Sk), v.dtype),
            pltpu.VMEM((Sq, D), q.dtype),
            pltpu.SemaphoreType.DMA((_LEAD,)),
            pltpu.SemaphoreType.DMA((_LEAD,)),
            pltpu.SemaphoreType.DMA((_LEAD,)),
            pltpu.SemaphoreType.DMA((2,)),
        ],
        compiler_params=pltpu.CompilerParams(
            vmem_limit_bytes=80 * 1024 * 1024,
            disable_bounds_checks=True,
            flags={"XLA_TPU_RESCHEDULE_DMA_DONES": True},
        ),
    )(qt, kt, vt)
    return jnp.swapaxes(ot.reshape(B, H, D, Sq), 2, 3)
```
